```python
import os as _os
_os.environ.setdefault("JAX_PLATFORMS", "cpu")
import jax
import jax.numpy as jnp

def _softmax(x, axis=-1):
    return jax.nn.softmax(x, axis=axis)
def _gelu(x):
    return jax.nn.gelu(x, approximate=True)
def _silu(x):
    return jax.nn.silu(x)
def _sigmoid(x):
    return jax.nn.sigmoid(x)
def _layernorm(x, axis=-1, eps=1e-5):
    m = jnp.mean(x, axis=axis, keepdims=True)
    v = jnp.var(x, axis=axis, keepdims=True)
    return (x - m) / jnp.sqrt(v + eps)
def _scatter_add(tgt, idx, src, axis=0):
    return tgt.at[idx].add(src)
def _segment_sum(src, seg, n):
    return jax.ops.segment_sum(src, seg, n)
class _Rng:
    def __init__(self, key):
        self._k = key
    def _next(self):
        self._k, sub = jax.random.split(self._k)
        return sub
    def normal(self, shape):
        return jax.random.normal(self._next(), shape, dtype=jnp.bfloat16)
    def randint(self, lo, hi, shape):
        return jax.random.randint(self._next(), shape, lo, hi, dtype=jnp.int32)
    def uniform(self, shape, lo=0.0, hi=1.0):
        return jax.random.uniform(self._next(), shape, jnp.bfloat16, lo, hi)
    def permutation(self, n):
        return jax.random.permutation(self._next(), n)


kernel_name = 'interleave_layers__spectral_gfnet__dense_activation_gelu__prompt'

def setup_inputs():
    _rng = _Rng(jax.random.key(int.from_bytes(__import__("os").urandom(4), "little")))
    _w = (lambda a: (lambda t: t.astype(jnp.bfloat16) if jnp.issubdtype(t.dtype, jnp.floating) else t)(jnp.asarray(a)))
    def _A_setup():
        B, S, D = 1, 2048, 640
        Df = D // 2 + 1
        return {
            "x": _w((lambda *s: _rng.normal(s) * 0.05)(B, S, D)),
            "w_r": _w((lambda *s: _rng.normal(s) * 0.2)(S, Df) * 0.02),
            "w_i": _w((lambda *s: _rng.normal(s) * 0.2)(S, Df) * 0.02),
        }
    _A_in = _A_setup()

    def _B_setup():
        B, S, D, F = 1, 2048, 640, 1728
        return {
            "x": _w((lambda *s: _rng.normal(s) * 0.05)(B, S, D)),
            "w1": _w((lambda *s: _rng.normal(s) * 0.1)(D, F) * (D ** -0.5)),
            "b1": _w((lambda *s: _rng.normal(s) * 0.1)(F) * 0.01),
            "w2": _w((lambda *s: _rng.normal(s) * 0.1)(F, D) * (F ** -0.5)),
            "b2": _w((lambda *s: _rng.normal(s) * 0.1)(D) * 0.01),
        }
    _B_in = _B_setup()

    return {
        "A_x": _A_in["x"],
        "A_w_r": _A_in["w_r"],
        "A_w_i": _A_in["w_i"],
        "B_x": _B_in["x"],
        "B_w1": _B_in["w1"],
        "B_b1": _B_in["b1"],
        "B_w2": _B_in["w2"],
        "B_b2": _B_in["b2"],
    }

def reference(A_x, A_w_r, A_w_i, B_x, B_w1, B_b1, B_w2, B_b2):
    def _A_ref(x, w_r, w_i):
        B, S, D = x.shape
        X = (lambda x, axes=(-2,-1): jnp.fft.rfft2(x.astype(jnp.float32), axes=axes))(x, axes=(-2, -1))
        W = w_r + 1j * w_i
        X = X * W
        y = (lambda x, s, axes=(-2,-1): jnp.fft.irfft2(x, s=s, axes=axes).astype(jnp.bfloat16))(X, (S, D), axes=(-2, -1))
        return y

    def _B_ref(x, w1, b1, w2, b2):
        h = jnp.einsum("bsd,df->bsf", x, w1) + b1
        h = _gelu(h)
        return jnp.einsum("bsf,fd->bsd", h, w2) + b2

    x = A_x
    x = x + _A_ref(_layernorm(x, axis=-1), A_w_r, A_w_i)
    x = x + _B_ref(_layernorm(x, axis=-1), B_w1, B_b1, B_w2, B_b2)
    x = x + _A_ref(_layernorm(x, axis=-1), A_w_r, A_w_i)
    x = x + _B_ref(_layernorm(x, axis=-1), B_w1, B_b1, B_w2, B_b2)
    return x
```

```python
import functools
import numpy as np
import jax
import jax.numpy as jnp
from jax import lax
import jax.experimental.pallas as pl
import jax.experimental.pallas.tpu as pltpu

R = 16
LANES = 128


def _round_up(a, b):
    return (a + b - 1) // b * b


@functools.lru_cache(maxsize=None)
def _dft_constants(S, D):
    Df = D // 2 + 1
    LP = _round_up(Df, LANES)
    Q = S // R
    d = np.arange(D)[:, None]
    l = np.arange(Df)[None, :]
    ang = 2 * np.pi * ((d * l) % D) / D
    cf = np.zeros((D, 2 * LP), np.float64)
    cf[:, :Df] = np.cos(ang)
    cf[:, LP:LP + Df] = -np.sin(ang)
    c = np.full(Df, 2.0)
    c[0] = 1.0
    c[-1] = 1.0
    ci = np.zeros((2 * LP, D), np.float64)
    ci[:Df, :] = c[:, None] * np.cos(ang.T) / (S * D)
    ci[LP:LP + Df, :] = -c[:, None] * np.sin(ang.T) / (S * D)
    j = np.arange(Q)
    g = np.zeros((R, 2 * Q, 2 * Q), np.float64)
    for a in range(R):
        th = 2 * np.pi * ((j[None, :] * (a + R * j[:, None])) % S) / S
        gr, gi = np.cos(th), -np.sin(th)
        g[a, :Q, :Q] = gr
        g[a, :Q, Q:] = -gi
        g[a, Q:, :Q] = gi
        g[a, Q:, Q:] = gr
    h = np.transpose(g, (0, 2, 1))
    bf = jnp.bfloat16
    return tuple(np.asarray(m).astype(bf) for m in (cf, ci, g, h))


def _fft_list(xs, sign):
    n = len(xs)
    if n == 1:
        return xs
    ev = _fft_list(xs[0::2], sign)
    od = _fft_list(xs[1::2], sign)
    out = [None] * n
    for k in range(n // 2):
        orr, oi = od[k]
        if k == 0:
            tr, ti = orr, oi
        elif 4 * k == n:
            tr, ti = (-oi, orr) if sign > 0 else (oi, -orr)
        else:
            c = float(np.cos(2 * np.pi * k / n))
            s = float(sign * np.sin(2 * np.pi * k / n))
            tr = orr * c - oi * s
            ti = orr * s + oi * c
        er, ei = ev[k]
        out[k] = (er + tr, ei + ti)
        out[k + n // 2] = (er - tr, ei - ti)
    return out


def _layernorm_bf16(x):
    bf = jnp.bfloat16
    xf = x.astype(jnp.float32)
    mean = jnp.mean(xf, axis=-1, keepdims=True)
    cen = xf - mean
    var = jnp.mean(cen * cen, axis=-1, keepdims=True)
    m = mean.astype(bf).astype(jnp.float32)
    v = var.astype(bf).astype(jnp.float32)
    dlt = (xf - m).astype(bf).astype(jnp.float32)
    den = jnp.sqrt((v + 1e-5).astype(bf).astype(jnp.float32)).astype(bf).astype(jnp.float32)
    return (dlt / den).astype(bf)


def _gelu_tanh(h):
    c = 0.7978845608028654
    return 0.5 * h * (1.0 + jnp.tanh(c * (h + 0.044715 * (h * h * h))))


def _make_kernel(S, D, F, TM):
    Df = D // 2 + 1
    LP = _round_up(Df, LANES)
    Q = S // R
    nblk = S // TM
    bf = jnp.bfloat16
    f32 = jnp.float32

    def kernel(x_ref, wr_ref, wi_ref, w1_ref, b1_ref, w2_ref, b2_ref,
               cf_ref, ci_ref, g_ref, h_ref, o_ref,
               xs, ybuf, tbuf, ubuf, rbuf, wrf, wif, wtmp):
        for src, dst in ((wr_ref, wrf), (wi_ref, wif)):
            for t in range(LP // LANES):
                lo = t * LANES
                n = min(LANES, Df - lo)
                if n < LANES:
                    wtmp[...] = jnp.zeros(wtmp.shape, f32)
                wtmp[:, 0:n] = src[:, lo:lo + n].astype(f32)
                for a in range(R):
                    dst[a, :, lo:lo + LANES] = wtmp[pl.ds(a, Q, stride=R), :]

        def dfwd(xblk, row0):
            y = jnp.dot(_layernorm_bf16(xblk), cf_ref[...], preferred_element_type=f32)
            ybuf[pl.ds(row0, TM), :] = y

        def vpu_fwd():
            def body(c, _):
                r0 = pl.multiple_of(c * 16, 16)
                for t in range(LP // LANES):
                    xs_ = [(ybuf[pl.ds(m * Q + r0, 16), pl.ds(t * LANES, LANES)],
                            ybuf[pl.ds(m * Q + r0, 16), pl.ds(LP + t * LANES, LANES)])
                           for m in range(R)]
                    out = _fft_list(xs_, -1)
                    for a in range(R):
                        tbuf[a, pl.ds(r0, 16), pl.ds(t * LANES, LANES)] = out[a][0].astype(bf)
                        tbuf[a, pl.ds(Q + r0, 16), pl.ds(t * LANES, LANES)] = out[a][1].astype(bf)
                return 0
            lax.fori_loop(0, Q // 16, body, 0)

        def mxu_mid():
            def body(a, _):
                z = jnp.dot(g_ref[a], tbuf[a], preferred_element_type=f32)
                zr, zi = z[:Q], z[Q:]
                wr = wrf[a]
                wi = wif[a]
                vr = zr * wr - zi * wi
                vi = zr * wi + zi * wr
                v = jnp.concatenate([vr, vi], axis=0).astype(bf)
                ubuf[a] = jnp.dot(h_ref[a], v, preferred_element_type=f32)
                return 0
            lax.fori_loop(0, R, body, 0)

        def vpu_inv():
            def body(c, _):
                r0 = pl.multiple_of(c * 16, 16)
                for t in range(LP // LANES):
                    xs_ = [(ubuf[a, pl.ds(r0, 16), pl.ds(t * LANES, LANES)],
                            ubuf[a, pl.ds(Q + r0, 16), pl.ds(t * LANES, LANES)])
                           for a in range(R)]
                    out = _fft_list(xs_, +1)
                    for m in range(R):
                        rbuf[pl.ds(m * Q + r0, 16), pl.ds(t * LANES, LANES)] = out[m][0].astype(bf)
                        rbuf[pl.ds(m * Q + r0, 16), pl.ds(LP + t * LANES, LANES)] = out[m][1].astype(bf)
                return 0
            lax.fori_loop(0, Q // 16, body, 0)

        def spectral():
            vpu_fwd()
            mxu_mid()
            vpu_inv()

        def dinv_mlp(xblk, row0):
            y = jnp.dot(rbuf[pl.ds(row0, TM), :], ci_ref[...], preferred_element_type=f32)
            x1 = xblk + y.astype(bf)
            hh = jnp.dot(_layernorm_bf16(x1), w1_ref[...], preferred_element_type=f32)
            hh = (hh.astype(bf) + b1_ref[...]).astype(f32)
            hh = _gelu_tanh(hh).astype(bf)
            y2 = jnp.dot(hh, w2_ref[...], preferred_element_type=f32)
            return x1 + (y2.astype(bf) + b2_ref[...])

        def p1(i, _):
            row0 = pl.multiple_of(i * TM, TM)
            dfwd(x_ref[pl.ds(row0, TM), :], row0)
            return 0
        lax.fori_loop(0, nblk, p1, 0)
        spectral()

        def p2(i, _):
            row0 = pl.multiple_of(i * TM, TM)
            x2 = dinv_mlp(x_ref[pl.ds(row0, TM), :], row0)
            xs[pl.ds(row0, TM), :] = x2
            dfwd(x2, row0)
            return 0
        lax.fori_loop(0, nblk, p2, 0)
        spectral()

        def p3(i, _):
            row0 = pl.multiple_of(i * TM, TM)
            o_ref[pl.ds(row0, TM), :] = dinv_mlp(xs[pl.ds(row0, TM), :], row0)
            return 0
        lax.fori_loop(0, nblk, p3, 0)

    scratch = [
        pltpu.VMEM((S, D), bf),
        pltpu.VMEM((S, 2 * LP), f32),
        pltpu.VMEM((R, 2 * Q, LP), bf),
        pltpu.VMEM((R, 2 * Q, LP), f32),
        pltpu.VMEM((S, 2 * LP), bf),
        pltpu.VMEM((R, Q, LP), f32),
        pltpu.VMEM((R, Q, LP), f32),
        pltpu.VMEM((S, LANES), f32),
    ]
    return kernel, scratch


@jax.jit
def pallas_interleave_layers__spectral_gfnet__dense_activation_gelu__prompt_kernel(
    A_x: jax.Array,
    A_w_r: jax.Array,
    A_w_i: jax.Array,
    B_x: jax.Array,
    B_w1: jax.Array,
    B_b1: jax.Array,
    B_w2: jax.Array,
    B_b2: jax.Array,
):
    B, S, D = A_x.shape
    F = B_w1.shape[1]
    assert B == 1
    TM = 256
    cf, ci, g, h = _dft_constants(S, D)
    kernel, scratch = _make_kernel(S, D, F, TM)
    vm = pl.BlockSpec(memory_space=pltpu.VMEM)
    out = pl.pallas_call(
        kernel,
        out_shape=jax.ShapeDtypeStruct((S, D), A_x.dtype),
        in_specs=[vm] * 11,
        out_specs=vm,
        scratch_shapes=scratch,
        compiler_params=pltpu.CompilerParams(vmem_limit_bytes=100 * 1024 * 1024),
    )(A_x.reshape(S, D), A_w_r, A_w_i, B_w1, B_b1.reshape(1, F), B_w2,
      B_b2.reshape(1, D), cf, ci, g, h)
    return out.reshape(B, S, D)
```

```python
import functools
import numpy as np
import jax
import jax.numpy as jnp
from jax import lax
import jax.experimental.pallas as pl
import jax.experimental.pallas.tpu as pltpu

R = 16
LANES = 128
SKIP = ''
UNROLL = 4
TM_ROWS = 256


def _round_up(a, b):
    return (a + b - 1) // b * b


@functools.lru_cache(maxsize=None)
def _dft_constants(S, D):
    Df = D // 2 + 1
    LP = _round_up(Df, LANES)
    Q = S // R
    d = np.arange(D)[:, None]
    l = np.arange(Df)[None, :]
    ang = 2 * np.pi * ((d * l) % D) / D
    cf = np.zeros((D, 2 * LP), np.float64)
    cf[:, :Df] = np.cos(ang)
    cf[:, LP:LP + Df] = -np.sin(ang)
    c = np.full(Df, 2.0)
    c[0] = 1.0
    c[-1] = 1.0
    ci = np.zeros((2 * LP, D), np.float64)
    ci[:Df, :] = c[:, None] * np.cos(ang.T) / (S * D)
    ci[LP:LP + Df, :] = -c[:, None] * np.sin(ang.T) / (S * D)
    j = np.arange(Q)
    g = np.zeros((R, 2 * Q, 2 * Q), np.float64)
    for a in range(R):
        th = 2 * np.pi * ((j[None, :] * (a + R * j[:, None])) % S) / S
        gr, gi = np.cos(th), -np.sin(th)
        g[a, :Q, :Q] = gr
        g[a, :Q, Q:] = -gi
        g[a, Q:, :Q] = gi
        g[a, Q:, Q:] = gr
    h = np.transpose(g, (0, 2, 1))
    bf = jnp.bfloat16
    return tuple(np.asarray(m).astype(bf) for m in (cf, ci, g, h))


def _fft_list(xs, sign):
    n = len(xs)
    if n == 1:
        return xs
    ev = _fft_list(xs[0::2], sign)
    od = _fft_list(xs[1::2], sign)
    out = [None] * n
    for k in range(n // 2):
        orr, oi = od[k]
        if k == 0:
            tr, ti = orr, oi
        elif 4 * k == n:
            tr, ti = (-oi, orr) if sign > 0 else (oi, -orr)
        else:
            c = float(np.cos(2 * np.pi * k / n))
            s = float(sign * np.sin(2 * np.pi * k / n))
            tr = orr * c - oi * s
            ti = orr * s + oi * c
        er, ei = ev[k]
        out[k] = (er + tr, ei + ti)
        out[k + n // 2] = (er - tr, ei - ti)
    return out


def _layernorm_bf16(x):
    bf = jnp.bfloat16
    xf = x.astype(jnp.float32)
    mean = jnp.mean(xf, axis=-1, keepdims=True)
    cen = xf - mean
    var = jnp.mean(cen * cen, axis=-1, keepdims=True)
    m = mean.astype(bf).astype(jnp.float32)
    v = var.astype(bf).astype(jnp.float32)
    dlt = (xf - m).astype(bf).astype(jnp.float32)
    den = jnp.sqrt((v + 1e-5).astype(bf).astype(jnp.float32)).astype(bf).astype(jnp.float32)
    return (dlt / den).astype(bf)


def _gelu_tanh(h):
    c = 0.7978845608028654
    return 0.5 * h * (1.0 + jnp.tanh(c * (h + 0.044715 * (h * h * h))))


def _make_kernel(S, D, F, TM):
    Df = D // 2 + 1
    LP = _round_up(Df, LANES)
    Q = S // R
    nblk = S // TM
    bf = jnp.bfloat16
    f32 = jnp.float32

    def kernel(x_ref, wr_ref, wi_ref, w1_ref, b1_ref, w2_ref, b2_ref,
               cf_ref, ci_ref, g_ref, h_ref, o_ref,
               xs, ybuf, tbuf, ubuf, rbuf, wrf, wif, wtmp):
        for src, dst in ((wr_ref, wrf), (wi_ref, wif)):
            for t in range(LP // LANES):
                lo = t * LANES
                n = min(LANES, Df - lo)
                if n < LANES:
                    wtmp[...] = jnp.zeros(wtmp.shape, f32)
                wtmp[:, 0:n] = src[:, lo:lo + n].astype(f32)
                for a in range(R):
                    dst[a, :, lo:lo + LANES] = wtmp[pl.ds(a, Q, stride=R), :]

        def dfwd(xblk, row0):
            y = jnp.dot(_layernorm_bf16(xblk), cf_ref[...], preferred_element_type=f32)
            ybuf[pl.ds(row0, TM), :] = y

        def vpu_fwd():
            def body(c, _):
                r0 = pl.multiple_of(c * 16, 16)
                for t in range(LP // LANES):
                    xs_ = [(ybuf[pl.ds(m * Q + r0, 16), pl.ds(t * LANES, LANES)],
                            ybuf[pl.ds(m * Q + r0, 16), pl.ds(LP + t * LANES, LANES)])
                           for m in range(R)]
                    out = _fft_list(xs_, -1)
                    for a in range(R):
                        tbuf[a, pl.ds(r0, 16), pl.ds(t * LANES, LANES)] = out[a][0].astype(bf)
                        tbuf[a, pl.ds(Q + r0, 16), pl.ds(t * LANES, LANES)] = out[a][1].astype(bf)
                return 0
            lax.fori_loop(0, Q // 16, body, 0)

        def mxu_mid():
            def body(a, _):
                z = jnp.dot(g_ref[a], tbuf[a], preferred_element_type=f32)
                zr, zi = z[:Q], z[Q:]
                wr = wrf[a]
                wi = wif[a]
                vr = zr * wr - zi * wi
                vi = zr * wi + zi * wr
                v = jnp.concatenate([vr, vi], axis=0).astype(bf)
                ubuf[a] = jnp.dot(h_ref[a], v, preferred_element_type=f32)
                return 0
            lax.fori_loop(0, R, body, 0, unroll=UNROLL)

        def vpu_inv():
            def body(c, _):
                r0 = pl.multiple_of(c * 16, 16)
                for t in range(LP // LANES):
                    xs_ = [(ubuf[a, pl.ds(r0, 16), pl.ds(t * LANES, LANES)],
                            ubuf[a, pl.ds(Q + r0, 16), pl.ds(t * LANES, LANES)])
                           for a in range(R)]
                    out = _fft_list(xs_, +1)
                    for m in range(R):
                        rbuf[pl.ds(m * Q + r0, 16), pl.ds(t * LANES, LANES)] = out[m][0].astype(bf)
                        rbuf[pl.ds(m * Q + r0, 16), pl.ds(LP + t * LANES, LANES)] = out[m][1].astype(bf)
                return 0
            lax.fori_loop(0, Q // 16, body, 0)

        def spectral():
            if SKIP != "vpu":
                vpu_fwd()
            if SKIP != "mxu":
                mxu_mid()
            if SKIP != "vpu":
                vpu_inv()

        def dinv_mlp(xblk, row0):
            y = jnp.dot(rbuf[pl.ds(row0, TM), :], ci_ref[...], preferred_element_type=f32)
            x1 = xblk + y.astype(bf)
            hh = lax.dot_general(_layernorm_bf16(x1), w1_ref[...], (((1,), (1,)), ((), ())),
                                 preferred_element_type=f32)
            hh = (hh.astype(bf) + b1_ref[...]).astype(f32)
            hh = _gelu_tanh(hh).astype(bf)
            y2 = jnp.dot(hh, w2_ref[...], preferred_element_type=f32)
            return x1 + (y2.astype(bf) + b2_ref[...])

        def p1(i, _):
            row0 = pl.multiple_of(i * TM, TM)
            dfwd(x_ref[pl.ds(row0, TM), :], row0)
            return 0
        lax.fori_loop(0, nblk, p1, 0)
        spectral()

        def p2(i, _):
            row0 = pl.multiple_of(i * TM, TM)
            x2 = dinv_mlp(x_ref[pl.ds(row0, TM), :], row0)
            xs[pl.ds(row0, TM), :] = x2
            dfwd(x2, row0)
            return 0
        lax.fori_loop(0, nblk, p2, 0)
        spectral()

        def p3(i, _):
            row0 = pl.multiple_of(i * TM, TM)
            o_ref[pl.ds(row0, TM), :] = dinv_mlp(xs[pl.ds(row0, TM), :], row0)
            return 0
        lax.fori_loop(0, nblk, p3, 0)

    scratch = [
        pltpu.VMEM((S, D), bf),
        pltpu.VMEM((S, 2 * LP), f32),
        pltpu.VMEM((R, 2 * Q, LP), bf),
        pltpu.VMEM((R, 2 * Q, LP), f32),
        pltpu.VMEM((S, 2 * LP), bf),
        pltpu.VMEM((R, Q, LP), f32),
        pltpu.VMEM((R, Q, LP), f32),
        pltpu.VMEM((S, LANES), f32),
    ]
    return kernel, scratch


@jax.jit
def pallas_interleave_layers__spectral_gfnet__dense_activation_gelu__prompt_kernel(
    A_x: jax.Array,
    A_w_r: jax.Array,
    A_w_i: jax.Array,
    B_x: jax.Array,
    B_w1: jax.Array,
    B_b1: jax.Array,
    B_w2: jax.Array,
    B_b2: jax.Array,
):
    B, S, D = A_x.shape
    F = B_w1.shape[1]
    assert B == 1
    TM = TM_ROWS
    cf, ci, g, h = _dft_constants(S, D)
    kernel, scratch = _make_kernel(S, D, F, TM)
    vm = pl.BlockSpec(memory_space=pltpu.VMEM)
    out = pl.pallas_call(
        kernel,
        out_shape=jax.ShapeDtypeStruct((S, D), A_x.dtype),
        in_specs=[vm] * 11,
        out_specs=vm,
        scratch_shapes=scratch,
        compiler_params=pltpu.CompilerParams(vmem_limit_bytes=100 * 1024 * 1024),
    )(A_x.reshape(S, D), A_w_r, A_w_i, B_w1.T, B_b1.reshape(1, F), B_w2,
      B_b2.reshape(1, D), cf, ci, g, h)
    return out.reshape(B, S, D)
```

```python
import functools
import numpy as np
import jax
import jax.numpy as jnp
from jax import lax
import jax.experimental.pallas as pl
import jax.experimental.pallas.tpu as pltpu

R = 16
LANES = 128
SKIP = ''
UNROLL = 4
TM_ROWS = 256


def _round_up(a, b):
    return (a + b - 1) // b * b


@functools.lru_cache(maxsize=None)
def _dft_constants(S, D):
    Df = D // 2 + 1
    LP = _round_up(Df, LANES)
    Q = S // R
    d = np.arange(D)[:, None]
    l = np.arange(Df)[None, :]
    ang = 2 * np.pi * ((d * l) % D) / D
    cf = np.zeros((D, 2 * LP), np.float64)
    cf[:, :Df] = np.cos(ang)
    cf[:, LP:LP + Df] = -np.sin(ang)
    c = np.full(Df, 2.0)
    c[0] = 1.0
    c[-1] = 1.0
    ci = np.zeros((2 * LP, D), np.float64)
    ci[:Df, :] = c[:, None] * np.cos(ang.T) / (S * D)
    ci[LP:LP + Df, :] = -c[:, None] * np.sin(ang.T) / (S * D)
    j = np.arange(Q)
    g = np.zeros((R, 2 * Q, 2 * Q), np.float64)
    for a in range(R):
        th = 2 * np.pi * ((j[None, :] * (a + R * j[:, None])) % S) / S
        gr, gi = np.cos(th), -np.sin(th)
        g[a, :Q, :Q] = gr
        g[a, :Q, Q:] = -gi
        g[a, Q:, :Q] = gi
        g[a, Q:, Q:] = gr
    h = np.transpose(g, (0, 2, 1))
    bf = jnp.bfloat16
    return tuple(np.asarray(m).astype(bf) for m in (cf, ci, g, h))


def _fft_list(xs, sign):
    n = len(xs)
    if n == 1:
        return xs
    ev = _fft_list(xs[0::2], sign)
    od = _fft_list(xs[1::2], sign)
    out = [None] * n
    for k in range(n // 2):
        orr, oi = od[k]
        if k == 0:
            tr, ti = orr, oi
        elif 4 * k == n:
            tr, ti = (-oi, orr) if sign > 0 else (oi, -orr)
        else:
            c = float(np.cos(2 * np.pi * k / n))
            s = float(sign * np.sin(2 * np.pi * k / n))
            tr = orr * c - oi * s
            ti = orr * s + oi * c
        er, ei = ev[k]
        out[k] = (er + tr, ei + ti)
        out[k + n // 2] = (er - tr, ei - ti)
    return out


def _layernorm_bf16(x):
    bf = jnp.bfloat16
    xf = x.astype(jnp.float32)
    mean = jnp.mean(xf, axis=-1, keepdims=True)
    cen = xf - mean
    var = jnp.mean(cen * cen, axis=-1, keepdims=True)
    m = mean.astype(bf).astype(jnp.float32)
    v = var.astype(bf).astype(jnp.float32)
    dlt = (xf - m).astype(bf).astype(jnp.float32)
    den = jnp.sqrt((v + 1e-5).astype(bf).astype(jnp.float32)).astype(bf).astype(jnp.float32)
    return (dlt / den).astype(bf)


def _gelu_tanh(h):
    c = 0.7978845608028654
    return 0.5 * h * (1.0 + jnp.tanh(c * (h + 0.044715 * (h * h * h))))


def _make_kernel(S, D, F, TM):
    Df = D // 2 + 1
    LP = _round_up(Df, LANES)
    Q = S // R
    nblk = S // TM
    bf = jnp.bfloat16
    f32 = jnp.float32

    def kernel(x_ref, wr_ref, wi_ref, w1_ref, b1_ref, w2_ref, b2_ref,
               cf_ref, ci_ref, g_ref, h_ref, o_ref,
               xs, ybuf, tbuf, ubuf, rbuf, wrf, wif, wtmp, w1s):
        w1s[...] = w1_ref[...].T
        for src, dst in ((wr_ref, wrf), (wi_ref, wif)):
            for t in range(LP // LANES):
                lo = t * LANES
                n = min(LANES, Df - lo)
                if n < LANES:
                    wtmp[...] = jnp.zeros(wtmp.shape, f32)
                wtmp[:, 0:n] = src[:, lo:lo + n].astype(f32)
                for a in range(R):
                    dst[a, :, lo:lo + LANES] = wtmp[pl.ds(a, Q, stride=R), :]

        def dfwd(xblk, row0):
            y = jnp.dot(_layernorm_bf16(xblk), cf_ref[...], preferred_element_type=f32)
            ybuf[pl.ds(row0, TM), :] = y

        def vpu_fwd():
            def body(c, _):
                r0 = pl.multiple_of(c * 16, 16)
                for t in range(LP // LANES):
                    xs_ = [(ybuf[pl.ds(m * Q + r0, 16), pl.ds(t * LANES, LANES)],
                            ybuf[pl.ds(m * Q + r0, 16), pl.ds(LP + t * LANES, LANES)])
                           for m in range(R)]
                    out = _fft_list(xs_, -1)
                    for a in range(R):
                        tbuf[a, pl.ds(r0, 16), pl.ds(t * LANES, LANES)] = out[a][0].astype(bf)
                        tbuf[a, pl.ds(Q + r0, 16), pl.ds(t * LANES, LANES)] = out[a][1].astype(bf)
                return 0
            lax.fori_loop(0, Q // 16, body, 0)

        def mxu_mid():
            def body(a, _):
                z = jnp.dot(g_ref[a], tbuf[a], preferred_element_type=f32)
                zr, zi = z[:Q], z[Q:]
                wr = wrf[a]
                wi = wif[a]
                vr = zr * wr - zi * wi
                vi = zr * wi + zi * wr
                v = jnp.concatenate([vr, vi], axis=0).astype(bf)
                ubuf[a] = jnp.dot(h_ref[a], v, preferred_element_type=f32)
                return 0
            lax.fori_loop(0, R, body, 0, unroll=UNROLL)

        def vpu_inv():
            def body(c, _):
                r0 = pl.multiple_of(c * 16, 16)
                for t in range(LP // LANES):
                    xs_ = [(ubuf[a, pl.ds(r0, 16), pl.ds(t * LANES, LANES)],
                            ubuf[a, pl.ds(Q + r0, 16), pl.ds(t * LANES, LANES)])
                           for a in range(R)]
                    out = _fft_list(xs_, +1)
                    for m in range(R):
                        rbuf[pl.ds(m * Q + r0, 16), pl.ds(t * LANES, LANES)] = out[m][0].astype(bf)
                        rbuf[pl.ds(m * Q + r0, 16), pl.ds(LP + t * LANES, LANES)] = out[m][1].astype(bf)
                return 0
            lax.fori_loop(0, Q // 16, body, 0)

        def spectral():
            if SKIP != "vpu":
                vpu_fwd()
            if SKIP != "mxu":
                mxu_mid()
            if SKIP != "vpu":
                vpu_inv()

        def dinv_mlp(xblk, row0):
            y = jnp.dot(rbuf[pl.ds(row0, TM), :], ci_ref[...], preferred_element_type=f32)
            x1 = xblk + y.astype(bf)
            hh = jnp.dot(_layernorm_bf16(x1), w1s[...], preferred_element_type=f32)
            hh = (hh.astype(bf) + b1_ref[...]).astype(f32)
            hh = _gelu_tanh(hh).astype(bf)
            y2 = jnp.dot(hh, w2_ref[...], preferred_element_type=f32)
            return x1 + (y2.astype(bf) + b2_ref[...])

        def p1(i, _):
            row0 = pl.multiple_of(i * TM, TM)
            dfwd(x_ref[pl.ds(row0, TM), :], row0)
            return 0
        lax.fori_loop(0, nblk, p1, 0)
        spectral()

        def p2(i, _):
            row0 = pl.multiple_of(i * TM, TM)
            x2 = dinv_mlp(x_ref[pl.ds(row0, TM), :], row0)
            xs[pl.ds(row0, TM), :] = x2
            dfwd(x2, row0)
            return 0
        lax.fori_loop(0, nblk, p2, 0)
        spectral()

        def p3(i, _):
            row0 = pl.multiple_of(i * TM, TM)
            o_ref[pl.ds(row0, TM), :] = dinv_mlp(xs[pl.ds(row0, TM), :], row0)
            return 0
        lax.fori_loop(0, nblk, p3, 0)

    scratch = [
        pltpu.VMEM((S, D), bf),
        pltpu.VMEM((S, 2 * LP), f32),
        pltpu.VMEM((R, 2 * Q, LP), bf),
        pltpu.VMEM((R, 2 * Q, LP), f32),
        pltpu.VMEM((S, 2 * LP), bf),
        pltpu.VMEM((R, Q, LP), f32),
        pltpu.VMEM((R, Q, LP), f32),
        pltpu.VMEM((S, LANES), f32),
        pltpu.VMEM((D, F), bf),
    ]
    return kernel, scratch


@jax.jit
def pallas_interleave_layers__spectral_gfnet__dense_activation_gelu__prompt_kernel(
    A_x: jax.Array,
    A_w_r: jax.Array,
    A_w_i: jax.Array,
    B_x: jax.Array,
    B_w1: jax.Array,
    B_b1: jax.Array,
    B_w2: jax.Array,
    B_b2: jax.Array,
):
    B, S, D = A_x.shape
    F = B_w1.shape[1]
    assert B == 1
    TM = TM_ROWS
    cf, ci, g, h = _dft_constants(S, D)
    kernel, scratch = _make_kernel(S, D, F, TM)
    vm = pl.BlockSpec(memory_space=pltpu.VMEM)
    out = pl.pallas_call(
        kernel,
        out_shape=jax.ShapeDtypeStruct((S, D), A_x.dtype),
        in_specs=[vm] * 11,
        out_specs=vm,
        scratch_shapes=scratch,
        compiler_params=pltpu.CompilerParams(vmem_limit_bytes=100 * 1024 * 1024),
    )(A_x.reshape(S, D), A_w_r, A_w_i, B_w1.T, B_b1.reshape(1, F), B_w2,
      B_b2.reshape(1, D), cf, ci, g, h)
    return out.reshape(B, S, D)
```

```python
import functools
import numpy as np
import jax
import jax.numpy as jnp
from jax import lax
import jax.experimental.pallas as pl
import jax.experimental.pallas.tpu as pltpu

R = 16
LANES = 128
UNROLL = 4
TM_ROWS = 256


def _round_up(a, b):
    return (a + b - 1) // b * b


@functools.lru_cache(maxsize=None)
def _dft_constants(S, D):
    Df = D // 2 + 1
    LP = _round_up(Df, LANES)
    Q = S // R
    d = np.arange(D)[:, None]
    l = np.arange(Df)[None, :]
    ang = 2 * np.pi * ((d * l) % D) / D
    cf = np.zeros((D, 2 * LP), np.float64)
    cf[:, :Df] = np.cos(ang)
    cf[:, LP:LP + Df] = -np.sin(ang)
    c = np.full(Df, 2.0)
    c[0] = 1.0
    c[-1] = 1.0
    ci = np.zeros((2 * LP, D), np.float64)
    ci[:Df, :] = c[:, None] * np.cos(ang.T) / (S * D)
    ci[LP:LP + Df, :] = -c[:, None] * np.sin(ang.T) / (S * D)
    j = np.arange(Q)
    g = np.zeros((R, 2 * Q, 2 * Q), np.float64)
    for a in range(R):
        th = 2 * np.pi * ((j[None, :] * (a + R * j[:, None])) % S) / S
        gr, gi = np.cos(th), -np.sin(th)
        g[a, :Q, :Q] = gr
        g[a, :Q, Q:] = -gi
        g[a, Q:, :Q] = gi
        g[a, Q:, Q:] = gr
    h = np.transpose(g, (0, 2, 1))
    bf = jnp.bfloat16
    return tuple(np.asarray(m).astype(bf) for m in (cf, ci, g, h))


def _fft_list(xs, sign):
    n = len(xs)
    if n == 1:
        return xs
    ev = _fft_list(xs[0::2], sign)
    od = _fft_list(xs[1::2], sign)
    out = [None] * n
    for k in range(n // 2):
        orr, oi = od[k]
        if k == 0:
            tr, ti = orr, oi
        elif 4 * k == n:
            tr, ti = (-oi, orr) if sign > 0 else (oi, -orr)
        else:
            c = float(np.cos(2 * np.pi * k / n))
            s = float(sign * np.sin(2 * np.pi * k / n))
            tr = orr * c - oi * s
            ti = orr * s + oi * c
        er, ei = ev[k]
        out[k] = (er + tr, ei + ti)
        out[k + n // 2] = (er - tr, ei - ti)
    return out


def _layernorm_bf16(x):
    bf = jnp.bfloat16
    xf = x.astype(jnp.float32)
    mean = jnp.mean(xf, axis=-1, keepdims=True)
    cen = xf - mean
    var = jnp.mean(cen * cen, axis=-1, keepdims=True)
    m = mean.astype(bf).astype(jnp.float32)
    v = var.astype(bf).astype(jnp.float32)
    dlt = (xf - m).astype(bf).astype(jnp.float32)
    den = jnp.sqrt((v + 1e-5).astype(bf).astype(jnp.float32)).astype(bf).astype(jnp.float32)
    return (dlt / den).astype(bf)


def _gelu_tanh(h):
    c = 0.7978845608028654
    return 0.5 * h * (1.0 + jnp.tanh(c * (h + 0.044715 * (h * h * h))))


def _make_kernel(S, D, F, TM):
    Df = D // 2 + 1
    LP = _round_up(Df, LANES)
    Q = S // R
    nblk = S // TM
    bf = jnp.bfloat16
    f32 = jnp.float32

    def kernel(x_ref, wr_ref, wi_ref, w1_ref, b1_ref, w2_ref, b2_ref,
               cf_ref, ci_ref, g_ref, h_ref, o_ref,
               xs, ybuf, tbuf, ubuf, rbuf, wrf, wif, wtmp, w1s):
        w1s[...] = w1_ref[...].T
        for src, dst in ((wr_ref, wrf), (wi_ref, wif)):
            for t in range(LP // LANES):
                lo = t * LANES
                n = min(LANES, Df - lo)
                if n < LANES:
                    wtmp[...] = jnp.zeros(wtmp.shape, f32)
                wtmp[:, 0:n] = src[:, lo:lo + n].astype(f32)
                for a in range(R):
                    dst[a, :, lo:lo + LANES] = wtmp[pl.ds(a, Q, stride=R), :]

        def dfwd(xblk, row0):
            y = jnp.dot(_layernorm_bf16(xblk), cf_ref[...], preferred_element_type=f32)
            ybuf[pl.ds(row0, TM), :] = y

        def vpu_fwd():
            def body(c, _):
                r0 = pl.multiple_of(c * 16, 16)
                for t in range(LP // LANES):
                    xs_ = [(ybuf[pl.ds(m * Q + r0, 16), pl.ds(t * LANES, LANES)],
                            ybuf[pl.ds(m * Q + r0, 16), pl.ds(LP + t * LANES, LANES)])
                           for m in range(R)]
                    out = _fft_list(xs_, -1)
                    for a in range(R):
                        tbuf[a, pl.ds(r0, 16), pl.ds(t * LANES, LANES)] = out[a][0].astype(bf)
                        tbuf[a, pl.ds(Q + r0, 16), pl.ds(t * LANES, LANES)] = out[a][1].astype(bf)
                return 0
            lax.fori_loop(0, Q // 16, body, 0)

        def mxu_mid():
            def body(a, _):
                z = jnp.dot(g_ref[a], tbuf[a], preferred_element_type=f32)
                zr, zi = z[:Q], z[Q:]
                wr = wrf[a]
                wi = wif[a]
                vr = zr * wr - zi * wi
                vi = zr * wi + zi * wr
                v = jnp.concatenate([vr, vi], axis=0).astype(bf)
                ubuf[a] = jnp.dot(h_ref[a], v, preferred_element_type=f32)
                return 0
            lax.fori_loop(0, R, body, 0, unroll=UNROLL)

        def vpu_inv():
            def body(c, _):
                r0 = pl.multiple_of(c * 16, 16)
                for t in range(LP // LANES):
                    xs_ = [(ubuf[a, pl.ds(r0, 16), pl.ds(t * LANES, LANES)],
                            ubuf[a, pl.ds(Q + r0, 16), pl.ds(t * LANES, LANES)])
                           for a in range(R)]
                    out = _fft_list(xs_, +1)
                    for m in range(R):
                        rbuf[pl.ds(m * Q + r0, 16), pl.ds(t * LANES, LANES)] = out[m][0].astype(bf)
                        rbuf[pl.ds(m * Q + r0, 16), pl.ds(LP + t * LANES, LANES)] = out[m][1].astype(bf)
                return 0
            lax.fori_loop(0, Q // 16, body, 0)

        def spectral():
            vpu_fwd()
            mxu_mid()
            vpu_inv()

        def dinv_mlp(xblk, row0):
            y = jnp.dot(rbuf[pl.ds(row0, TM), :], ci_ref[...], preferred_element_type=f32)
            x1 = xblk + y.astype(bf)
            hh = jnp.dot(_layernorm_bf16(x1), w1s[...], preferred_element_type=f32)
            hh = (hh.astype(bf) + b1_ref[...]).astype(f32)
            hh = _gelu_tanh(hh).astype(bf)
            y2 = jnp.dot(hh, w2_ref[...], preferred_element_type=f32)
            return x1 + (y2.astype(bf) + b2_ref[...])

        def p1(i, _):
            row0 = pl.multiple_of(i * TM, TM)
            dfwd(x_ref[pl.ds(row0, TM), :], row0)
            return 0
        lax.fori_loop(0, nblk, p1, 0)
        spectral()

        def p2(i, _):
            row0 = pl.multiple_of(i * TM, TM)
            x2 = dinv_mlp(x_ref[pl.ds(row0, TM), :], row0)
            xs[pl.ds(row0, TM), :] = x2
            dfwd(x2, row0)
            return 0
        lax.fori_loop(0, nblk, p2, 0)
        spectral()

        def p3(i, _):
            row0 = pl.multiple_of(i * TM, TM)
            o_ref[pl.ds(row0, TM), :] = dinv_mlp(xs[pl.ds(row0, TM), :], row0)
            return 0
        lax.fori_loop(0, nblk, p3, 0)

    scratch = [
        pltpu.VMEM((S, D), bf),
        pltpu.VMEM((S, 2 * LP), f32),
        pltpu.VMEM((R, 2 * Q, LP), bf),
        pltpu.VMEM((R, 2 * Q, LP), f32),
        pltpu.VMEM((S, 2 * LP), bf),
        pltpu.VMEM((R, Q, LP), f32),
        pltpu.VMEM((R, Q, LP), f32),
        pltpu.VMEM((S, LANES), f32),
        pltpu.VMEM((D, F), bf),
    ]
    return kernel, scratch


@jax.jit
def pallas_interleave_layers__spectral_gfnet__dense_activation_gelu__prompt_kernel(
    A_x: jax.Array,
    A_w_r: jax.Array,
    A_w_i: jax.Array,
    B_x: jax.Array,
    B_w1: jax.Array,
    B_b1: jax.Array,
    B_w2: jax.Array,
    B_b2: jax.Array,
):
    B, S, D = A_x.shape
    F = B_w1.shape[1]
    assert B == 1
    TM = TM_ROWS
    cf, ci, g, h = _dft_constants(S, D)
    kernel, scratch = _make_kernel(S, D, F, TM)
    vm = pl.BlockSpec(memory_space=pltpu.VMEM)
    out = pl.pallas_call(
        kernel,
        out_shape=jax.ShapeDtypeStruct((S, D), A_x.dtype),
        in_specs=[vm] * 11,
        out_specs=vm,
        scratch_shapes=scratch,
        compiler_params=pltpu.CompilerParams(vmem_limit_bytes=100 * 1024 * 1024),
    )(A_x.reshape(S, D), A_w_r, A_w_i, B_w1.T, B_b1.reshape(1, F), B_w2,
      B_b2.reshape(1, D), cf, ci, g, h)
    return out.reshape(B, S, D)
```
